```python
import jax
import jax.numpy as jnp

def _softmax(x, axis=-1):
    return jax.nn.softmax(x, axis=axis)

def _gelu(x):
    return jax.nn.gelu(x, approximate=True)

def _silu(x):
    return jax.nn.silu(x)

def _sigmoid(x):
    return jax.nn.sigmoid(x)

def _layernorm(x, axis=-1, eps=1e-05):
    m = jnp.mean(x, axis=axis, keepdims=True)
    v = jnp.var(x, axis=axis, keepdims=True)
    return (x - m) / jnp.sqrt(v + eps)

def _scatter_add(tgt, idx, src, axis=0):
    return tgt.at[idx].add(src)

def _segment_sum(src, seg, n):
    return jax.ops.segment_sum(src, seg, n)

class _Rng:

    def __init__(self, key):
        self._k = key

    def _next(self):
        self._k, sub = jax.random.split(self._k)
        return sub

    def normal(self, shape):
        return jax.random.normal(self._next(), shape, dtype=jnp.bfloat16)

    def randint(self, lo, hi, shape):
        return jax.random.randint(self._next(), shape, lo, hi, dtype=jnp.int32)

    def uniform(self, shape, lo=0.0, hi=1.0):
        return jax.random.uniform(self._next(), shape, jnp.bfloat16, lo, hi)

    def permutation(self, n):
        return jax.random.permutation(self._next(), n)
kernel_name = 'adaLN_cond__grouped_kv_mqa__dense_activation_silu__prompt'

def _fwd_setup_inputs():
    _rng = _Rng(jax.random.key(int.from_bytes(__import__("os").urandom(4), "little")))
    _w = lambda a: (lambda t: t.astype(jnp.bfloat16) if jnp.issubdtype(t.dtype, jnp.floating) else t)(jnp.asarray(a))

    def _A_setup():
        B, S, D, H = (1, 2048, 640, 32)
        Dh = D // H
        return {'x': _w((lambda *s: _rng.normal(s) * 0.05)(B, S, D)), 'wq': _w((lambda *s: _rng.normal(s) * 0.05)(D, H * Dh)), 'wk': _w((lambda *s: _rng.normal(s) * 0.05)(D, Dh)), 'wv': _w((lambda *s: _rng.normal(s) * 0.05)(D, Dh)), 'wo': _w((lambda *s: _rng.normal(s) * 0.05)(H * Dh, D))}
    _A_in = _A_setup()

    def _B_setup():
        B, S, D, F = (1, 2048, 640, 1728)
        return {'x': _w((lambda *s: _rng.normal(s) * 0.05)(B, S, D)), 'w1': _w((lambda *s: _rng.normal(s) * 0.05)(D, F) * D ** (-0.5)), 'w2': _w((lambda *s: _rng.normal(s) * 0.05)(F, D) * F ** (-0.5))}
    _B_in = _B_setup()
    return {'A_x': _A_in['x'], 'A_wq': _A_in['wq'], 'A_wk': _A_in['wk'], 'A_wv': _A_in['wv'], 'A_wo': _A_in['wo'], 'B_x': _B_in['x'], 'B_w1': _B_in['w1'], 'B_w2': _B_in['w2'], 'c': _w((lambda *s: _rng.normal(s) * 0.05)(1, 640)), 'w_mod': _w((lambda *s: _rng.normal(s) * 0.05)(640, 6 * 640) * 640 ** (-0.5))}

def _fwd_reference(A_x, A_wq, A_wk, A_wv, A_wo, B_x, B_w1, B_w2, c, w_mod):

    def _A_ref(x, wq, wk, wv, wo):
        B, S, D = x.shape
        H = 32
        Dh = D // H
        q = (lambda x, *d: x.transpose(*d))((x @ wq).reshape(B, S, H, Dh), 0, 2, 1, 3)
        k = x @ wk
        v = x @ wv
        scores = jnp.einsum('bhqd,bkd->bhqk', q, k) * Dh ** (-0.5)
        p = _softmax(scores, axis=-1)
        o = jnp.einsum('bhqk,bkd->bhqd', p, v)
        return (lambda x, *d: x.transpose(*d))(o, 0, 2, 1, 3).reshape(B, S, H * Dh) @ wo

    def _B_ref(x, w1, w2):
        h = jnp.einsum('bsd,df->bsf', x, w1)
        h = _silu(h)
        out = jnp.einsum('bsf,fd->bsd', h, w2)
        return out
    x = A_x
    mod = (_silu(c) @ w_mod).reshape(c.shape[0], 6, 1, -1)
    sa, ca, ga, sb, cb, gb = (mod[:, 0].copy(), mod[:, 1].copy(), mod[:, 2].copy(), mod[:, 3].copy(), mod[:, 4].copy(), mod[:, 5].copy())
    h = _layernorm(x, axis=-1) * (1 + ca) + sa
    x = x + ga * _A_ref(h, A_wq, A_wk, A_wv, A_wo)
    h = _layernorm(x, axis=-1) * (1 + cb) + sb
    x = x + gb * _B_ref(h, B_w1, B_w2)
    return x

def setup_inputs():
    _inp = _fwd_setup_inputs()
    _gk = jax.random.fold_in(jax.random.key(int.from_bytes(__import__("os").urandom(4), "little")), 2 ** 31 - 1)
    _shapes = [[1, 2048, 640]]
    _dtypes = ['bfloat16']
    _gks = jax.random.split(_gk, len(_shapes))
    _gs = [jax.random.normal(k, s, dtype=jnp.dtype(d)) * 0.05 for k, s, d in zip(_gks, _shapes, _dtypes)]
    _inp['grad_out'] = _gs[0]
    return _inp

def reference(A_x, A_wq, A_wk, A_wv, A_wo, B_w1, B_w2, c, w_mod, B_x, grad_out):
    _const = dict(B_x=B_x)

    def _f(*_d):
        return _fwd_reference(**{'A_x': _d[0], 'A_wq': _d[1], 'A_wk': _d[2], 'A_wv': _d[3], 'A_wo': _d[4], 'B_w1': _d[5], 'B_w2': _d[6], 'c': _d[7], 'w_mod': _d[8], **_const})
    _out, _vjp = jax.vjp(_f, A_x, A_wq, A_wk, A_wv, A_wo, B_w1, B_w2, c, w_mod)
    _grads = _vjp(grad_out)
    _out0 = jnp.asarray(_out)
    return (_out0, *[jnp.asarray(_g) for _g in _grads])
```

```python
import math

import jax
import jax.numpy as jnp
import jax.experimental.pallas as pl
import jax.experimental.pallas.tpu as pltpu

F32 = jnp.float32
BF16 = jnp.bfloat16

N_HEADS = 32
EPS = 1e-5
SAFE_SCORE = 48.0
BQ = 256
CK = 128
DP = 24
FWD_UNROLL = 4
BWD_UNROLL = 4

VPU_KEYS = 16
AHEAD_KEYS = 8

FWD_PINS = {("out", 0): 13, ("out", 1): 19, ("out", 4): 25, ("out", 9): 32}
BWD_PINS = {("prev", 13): 8, ("lhs", 10): 12, ("lhs", 12): 16,
            ("out", 0): 20, ("out", 4): 24, ("out", 7): 29, ("out", 13): 32}
AHEAD_PLAN = dict(dg=4, a=2, u=12, dw2=30, dh2=14, mlp=15, do=7, dw1=24, dwo=12)
AHEAD_PIECES = 14
Q_CUTS = (160, 400)
DG_CUTS = (256, 768, 1344)
DW_SPLIT = 128
DW_CUTS = (128, 336)

_NN = (((1,), (0,)), ((), ()))
_NT = (((1,), (1,)), ((), ()))
_TN = (((0,), (0,)), ((), ()))


def _dot(a, b, dims=_NN):
    return jax.lax.dot_general(a, b, dims, preferred_element_type=F32)


def _rowsum8(v):
    return jnp.sum(v.reshape(v.shape[0] // 8, 8, v.shape[1]), axis=0)


def _sigmoid(v):
    return 0.5 * jnp.tanh(0.5 * v) + 0.5


def _fold(v):
    return sum(v[:, c:c + 128] for c in range(0, v.shape[1], 128))


def _row_mean(v, stages):
    folded = _fold(v)
    stages.append(folded)
    return jnp.sum(folded, axis=-1, keepdims=True) * (1.0 / v.shape[1])


def _layernorm(v, stages=None):
    stages = [] if stages is None else stages
    cen = v - _row_mean(v, stages)
    rstd = jax.lax.rsqrt(_row_mean(cen * cen, stages) + EPS)
    return cen * rstd, rstd


def _layernorm_bwd(dy, y, rstd):
    return (dy - _row_mean(dy, []) - y * _row_mean(dy * y, [])) * rstd


def _split_rows(row):
    hi = row.astype(BF16).astype(F32)
    mid = (row - hi).astype(BF16).astype(F32)
    return jnp.concatenate([hi, mid, row - hi - mid, row], axis=0)


def _regs(x):
    words = x if x.dtype == F32 else pltpu.bitcast(x, jnp.int32)
    return [[words[r:r + 8, c:c + 128] for c in range(0, words.shape[1], 128)]
            for r in range(0, words.shape[0], 8)]


def _pin(x, never, columns):
    regs = _regs(x)
    for c, groups in enumerate(columns):
        for i, group in enumerate(groups):
            r = (2 * i + 1) * len(regs) // (2 * len(groups))
            for part in group:
                if part.dtype != regs[r][c].dtype:
                    part = pltpu.bitcast(part, regs[r][c].dtype)
                regs[r][c] = jnp.where(never, part, regs[r][c])
    words = jnp.concatenate([jnp.concatenate(row, axis=1) for row in regs], axis=0)
    return words if x.dtype == F32 else pltpu.bitcast(words, x.dtype)


def _pin_value(x, never, value, rows):
    if not rows:
        return x
    regs = _regs(value)
    bands = [sum(regs[r:r + rows], []) for r in range(0, len(regs), rows)]
    n_c = x.shape[1] // 128
    return _pin(x, never, [bands[c::n_c] for c in range(n_c)])


class _VpuRows:
    def __init__(self, tab_ref, rhs_ref, g, j, never=None, pins=None):
        self.tab_ref, self.rhs_ref, self.g, self.j = tab_ref, rhs_ref, g, j
        self.never, self.pins = never, pins or {}
        self.depth = tab_ref.shape[1]
        self.acc = [None] * (rhs_ref.shape[2] // 128)
        self.done = 0

    def _tiles(self, step):
        n = len(self.acc) // 2
        return range(step // self.depth * n, (step // self.depth + 1) * n)

    def _advance(self, steps):
        for step in range(self.done, steps):
            e = step % self.depth
            col = self.tab_ref[self.j, e]
            for t in self._tiles(step):
                lanes = pl.ds(128 * t, 128)
                row = self.rhs_ref[self.g, e:e + 1, lanes]
                base = self.acc[t] if e else self.rhs_ref[self.g, DP - 1:DP, lanes]
                self.acc[t] = base + col * row
        self.done = max(self.done, steps)

    def partial(self, steps):
        self._advance(steps)
        return [self.acc[t][r:r + 8] for r in range(0, VPU_KEYS, 8)
                for t in self._tiles(steps - 1)]

    def pin(self, name, x):
        parts = [x[r:r + 8] for r in range(0, x.shape[0], 8)]
        for (where, i), steps in self.pins.items():
            if where == name:
                sums = self.partial(steps)
                if x.shape[1] == self.never.shape[1]:
                    sums = [jnp.concatenate(sums, axis=1)]
                for s in sums:
                    parts[i] = jnp.where(self.never[:, :x.shape[1]], s[:, :x.shape[1]],
                                         parts[i])
        return jnp.concatenate(parts, axis=0)

    def result(self):
        self._advance(2 * self.depth)
        return jnp.concatenate(self.acc, axis=1)


def _kernel(
    x_hbm, wq_hbm, wkt_hbm, wvt_hbm, wo_hbm, w1t_hbm, w2_hbm, c_hbm, wmod_hbm, dout_hbm,
    out_hbm, dx_hbm, dwq_hbm, dwkt_hbm, dwvt_hbm, dwo_hbm, dw1t_hbm, dw2_hbm, dc_hbm, dwmod_hbm,
    wkt_v, wvt_v, dwkt_s, dwvt_s, c_v, dc_s,
    x_v, dout_v, wq_v, wo_v, w1t_v, w2_v, wmod_v,
    wkv32, mod_v, dmod_acc, dwt_acc, wt_v, h_v, k_v, v_v, kt_v, vt_v,
    kb_v, kpre_v, vb_v, pre_v, norm_v, siluc_v,
    qt_v, dot_v, pv_v, dm_v, dqt_v, s_v, p_v, ds_v,
    dx_acc, dkt_acc, dvt_acc,
    dwo_acc, dw1t_acc, dw2_acc,
    dsilu_v, dwo_s, dw1t_s, dw2_s,
    in_sem, x_sem, out_sem, dx_sem, mod_sem, w_sem,
):
    out_s, dx_s, dwq_s, dwmod_s = dout_v, x_v, wq_v, wmod_v
    dmod_acc = dmod_acc.at[0:8]
    seq, d = x_v.shape
    dh = d // N_HEADS
    n_blk = seq // BQ
    n_grp = N_HEADS // 2
    n_chunk = seq // CK
    scale = dh ** -0.5
    q_scale = scale * math.log2(math.e)

    def rows(b):
        if isinstance(b, int):
            return pl.ds(b * BQ, BQ)
        return pl.ds(pl.multiple_of(b * BQ, BQ), BQ)

    def pair_rows(g):
        if isinstance(g, int):
            return pl.ds(g * 2 * dh, 2 * dh)
        return pl.ds(pl.multiple_of(g * 2 * dh, 8), 2 * dh)

    def keys(j):
        return pl.ds(j * CK, CK)

    def never_mask(i):
        return jnp.full((8, 2 * BQ), i, jnp.int32) < -1

    def modrow(i):
        return mod_v[0:1, i * d:(i + 1) * d]

    early = 2 * d
    cp_c = pltpu.make_async_copy(c_hbm, c_v.at[:, pl.ds(0, d)], in_sem.at[0])
    cp_wmod_a = pltpu.make_async_copy(
        wmod_hbm.at[:, pl.ds(0, early)], wmod_v.at[:, pl.ds(0, early)], in_sem.at[1])
    cp_wk = pltpu.make_async_copy(wkt_hbm, wkt_v, in_sem.at[2])
    cp_wv = pltpu.make_async_copy(wvt_hbm, wvt_v, in_sem.at[3])
    cp_wq = pltpu.make_async_copy(wq_hbm, wq_v, in_sem.at[4])
    cp_wmod_b = pltpu.make_async_copy(
        wmod_hbm.at[:, pl.ds(early, 4 * d)], wmod_v.at[:, pl.ds(early, 4 * d)], in_sem.at[5])
    cp_late = [
        pltpu.make_async_copy(dout_hbm, dout_v, in_sem.at[6]),
        pltpu.make_async_copy(wo_hbm, wo_v, in_sem.at[7]),
        pltpu.make_async_copy(w1t_hbm, w1t_v, in_sem.at[8]),
        pltpu.make_async_copy(w2_hbm, w2_v, in_sem.at[9]),
    ]

    def cp_x(b):
        return pltpu.make_async_copy(x_hbm.at[rows(b)], x_v.at[rows(b)], x_sem.at[b])

    def cp_out(b):
        return pltpu.make_async_copy(out_s.at[rows(b)], out_hbm.at[rows(b)], out_sem.at[b])

    def cp_dx(b):
        return pltpu.make_async_copy(dx_s.at[rows(b)], dx_hbm.at[rows(b)], dx_sem.at[b])

    def last_parts(i):
        quarter, strip = i * (d // 4), DW_SPLIT + i * 128
        if not isinstance(i, int):
            quarter, strip = pl.multiple_of(quarter, 16), pl.multiple_of(strip, 128)
        return pl.ds(quarter, d // 4), pl.ds(strip, 128)

    def cp_last(i):
        quarter, strip = last_parts(i)
        idx = (quarter, pl.ds(0, early))
        return [
            pltpu.make_async_copy(dwmod_s.at[idx], dwmod_hbm.at[idx], w_sem.at[7 + 2 * i]),
            pltpu.make_async_copy(dwq_s.at[:, strip], dwq_hbm.at[:, strip],
                                  w_sem.at[8 + 2 * i]),
        ]

    cp_w_early = [
        pltpu.make_async_copy(dwo_s, dwo_hbm, w_sem.at[0]),
        pltpu.make_async_copy(dw1t_s, dw1t_hbm, w_sem.at[1]),
        pltpu.make_async_copy(dw2_s, dw2_hbm, w_sem.at[2]),
    ]
    cp_w_late = [
        pltpu.make_async_copy(dwkt_s, dwkt_hbm, w_sem.at[3]),
        pltpu.make_async_copy(dwvt_s, dwvt_hbm, w_sem.at[4]),
    ]
    cp_w_last = [
        pltpu.make_async_copy(dc_s.at[:, pl.ds(0, d)], dc_hbm, w_sem.at[5]),
        pltpu.make_async_copy(dwq_s.at[:, pl.ds(0, DW_SPLIT)],
                              dwq_hbm.at[:, pl.ds(0, DW_SPLIT)], w_sem.at[6]),
    ]

    def mod_rows(b):
        n = d // n_blk
        return pl.ds(b * n if isinstance(b, int) else pl.multiple_of(b * n, 16), n)

    def cp_dwmod(b):
        idx = (mod_rows(b), pl.ds(early, 4 * d))
        return pltpu.make_async_copy(dwmod_s.at[idx], dwmod_hbm.at[idx], mod_sem.at[b])

    for cp in (cp_wq, cp_c, cp_wk, cp_wv, cp_x(0), cp_wmod_a, cp_x(1)):
        cp.start()

    def clear(i, carry):
        for ref in (dkt_acc, dvt_acc):
            ref[:, rows(i)] = jnp.zeros((DP, BQ), F32)
        for ref in (dwo_acc, dw1t_acc, dw2_acc, dwt_acc):
            n = ref.shape[0] // n_blk
            ref[pl.ds(pl.multiple_of(i * n, 8), n), :] = jnp.zeros((n, d), F32)
        return carry

    jax.lax.fori_loop(0, n_blk, clear, 0)
    for ref in (dmod_acc, norm_v, wkv32):
        ref[...] = jnp.zeros(ref.shape, ref.dtype)
    for cp in (cp_wq, cp_c, cp_wk, cp_wv, cp_x(0)):
        cp.wait()

    wkv32[0:dh, :] = wkt_v[...].astype(F32)
    wkv32[DP:DP + dh, :] = wvt_v[...].astype(F32)
    wt_v[0:d, :] = wq_v[...].T
    dx_acc[rows(0), :] = _layernorm(x_v[rows(0), :].astype(F32))[0]
    wt_v[d:d + 2 * DP, :] = wkv32[...].astype(BF16)
    c32 = jnp.broadcast_to(c_v[:, 0:d].astype(F32), (8, d))
    sig_c = _sigmoid(c32)
    silu_c = c32 * sig_c
    siluc_v[...] = jnp.broadcast_to(silu_c[0:1], (128, d)).T
    cp_wmod_a.wait()
    for b in range(2, n_blk):
        cp_x(b).start()
    mod_v[:, 0:early] = _dot(silu_c, wmod_v[:, 0:early])

    def modulate(b, stages=None):
        xhat, _ = _layernorm(x_v[rows(b), :].astype(F32), stages)
        return (xhat * (1.0 + modrow(1)) + modrow(0)).astype(BF16)

    def project(b, carry):
        @pl.when(b + 1 < n_blk)
        def _():
            cp_x(b + 1).wait()

        @pl.when(b == 1)
        def _():
            cp_wmod_b.start()

        h = h_v[rows(b), :]
        never = never_mask(b)[:, 0:128]
        b_next, stages = jnp.minimum(b + 1, n_blk - 1), []
        h_next = modulate(b_next, stages)
        h_v[rows(b_next), :] = h_next
        lo, hi = Q_CUTS
        last = _dot(_pin_value(wt_v[hi:d + 2 * DP, :], never, stages[1], 32), h, _NT)
        mid = _dot(_pin_value(wt_v[lo:hi, :], never, h_next, 1), h, _NT)
        first = _dot(wt_v[0:lo, :], h, _NT)
        kvt = last[d - hi:].astype(BF16).astype(F32)
        qt = jnp.concatenate([first, mid, last[:d - hi]], axis=0) * q_scale
        qt = qt.astype(BF16).astype(F32)
        tail = jnp.zeros((DP - dh, BQ), F32)
        q_norm = norm_v[0:1, :]
        for hd in range(N_HEADS):
            q = jnp.concatenate([qt[hd * dh:(hd + 1) * dh], tail], axis=0)
            qt_v[b * n_grp + hd // 2, :, pl.ds((hd % 2) * BQ, BQ)] = q
            q_norm = jnp.maximum(q_norm, jnp.sum(q * q, axis=0, keepdims=True))
        norm_v[0:1, :] = q_norm
        norm_v[8:9, :] = jnp.maximum(
            norm_v[8:9, :], jnp.sum(kvt[0:DP] * kvt[0:DP], axis=0, keepdims=True))
        r = jax.lax.broadcasted_iota(jnp.int32, (DP, BQ), 0)
        ones = jnp.where(r < dh + 3, 1.0, 0.0)
        kt = jnp.where(r < dh, kvt[0:DP], ones)
        vt = jnp.where(r < dh, kvt[DP:2 * DP], ones)
        kt_v[:, rows(b)] = kt
        vt_v[:, rows(b)] = vt
        pad = jnp.zeros((128 - DP, BQ), F32)
        k = jnp.concatenate([kt, pad], axis=0).T
        v = jnp.concatenate([vt, pad], axis=0).T
        k_v[rows(b), :] = k[:, 0:DP]
        v_v[rows(b), :] = v[:, 0:DP]
        for nat, tab_ref in ((k, kb_v), (v[CK - VPU_KEYS:], vb_v)):
            n = tab_ref.shape[2]
            for i in range(BQ // CK):
                for e in range(dh):
                    tab_ref[b * (BQ // CK) + i, e] = jnp.broadcast_to(
                        nat[i * CK:i * CK + n, e:e + 1], (n, 128))
        return carry

    h_v[rows(0), :] = (dx_acc[rows(0), :] * (1.0 + modrow(1)) + modrow(0)).astype(BF16)
    jax.lax.fori_loop(0, n_blk, project, 0)

    bound_sq = jnp.max(norm_v[0:1, :]) * jnp.max(norm_v[8:9, :])

    @pl.when(jnp.logical_not(bound_sq <= SAFE_SCORE ** 2))
    def _():
        def true_max(g, carry):
            def chunk(j, m):
                part = pl.ds(pl.multiple_of(j * CK, CK), CK)
                sc = _dot(k_v[part, :], qt_v[g])
                return jnp.maximum(m, jnp.max(sc.reshape(CK // 8, 8, 2 * BQ), axis=0))

            m = jax.lax.fori_loop(
                0, n_chunk, chunk, jnp.full((8, 2 * BQ), -jnp.inf, F32))
            qt_v[g, dh:DP, :] = _split_rows(-jnp.max(m, axis=0, keepdims=True))
            return carry

        jax.lax.fori_loop(0, n_blk * n_grp, true_max, 0)

    def fwd_steps(g0, slots, g0_next=None, never=None):
        acc = None
        for u in slots:
            g = g0 + u
            for j in range(n_chunk):
                own = pl.ds(j * CK, CK - AHEAD_KEYS)
                ahead = pl.ds(j * AHEAD_KEYS, AHEAD_KEYS)
                p = jnp.concatenate([jnp.exp2(s_v[u, own, :]), pre_v[g, ahead, :]], axis=0)
                if g0_next is not None:
                    vpu = _VpuRows(kb_v, qt_v, g0_next + u, j, never, FWD_PINS)
                    k = k_v[pl.ds(j * CK + VPU_KEYS, CK - AHEAD_KEYS - VPU_KEYS), :]
                    mxu = vpu.pin("out", _dot(k, qt_v[g0_next + u]))
                    s_v[u, own, :] = jnp.concatenate([vpu.result(), mxu], axis=0)
                p_v[g, keys(j), :] = p.astype(BF16)
                o = _dot(vt_v[:, keys(j)], p)
                if j:
                    acc = acc + o
                else:
                    acc = o if acc is None else jnp.where(never[0:1], acc, o)
            pv_v[g] = acc

    def gate_dout(b):
        dm_v[...] = (dout_v[rows(b), :].astype(F32) * modrow(5)).astype(BF16)

    def dscores(vpu, vpu_next):
        v = vpu.pin("lhs", v_v[pl.ds(vpu.j * CK, CK - VPU_KEYS), :])
        if vpu_next is not None:
            v = vpu_next.pin("prev", v)
        mxu = vpu.pin("out", _dot(v, dot_v[vpu.g]))
        dp = jnp.concatenate([mxu, vpu.result()], axis=0)
        return (p_v[vpu.g, keys(vpu.j), :].astype(F32) * dp).astype(BF16)

    def bwd_steps(b, g0, never):
        order = [(u, j) for j in range(n_chunk) for u in range(BWD_UNROLL)]
        items = [(g0 + u, j) for u, j in order]
        ahead = items[1:] + [(jnp.minimum(g0 + BWD_UNROLL, n_grp - 1), 0)]
        vpus = [_VpuRows(vb_v, dot_v, g, j, never, BWD_PINS if i else None)
                for i, (g, j) in enumerate(ahead)]
        ds = ds_v[...]
        acc = [None] * BWD_UNROLL
        for (u, j), vpu, vpu_next in zip(order, vpus, vpus[1:] + [None]):
            g = g0 + u
            ds_next = dscores(vpu, vpu_next)
            dvt_acc[:, keys(j)] += _dot(dot_v[g], p_v[g, keys(j), :], _NT)
            dkt_acc[:, keys(j)] += _dot(qt_v[b * n_grp + g], ds, _NT)
            dq = _dot(kt_v[:, keys(j)], ds)
            acc[u] = acc[u] + dq if j else dq
            if j == n_chunk - 1:
                dq = acc[u][0:dh] * scale
                dqt_v[pair_rows(g), rows(b)] = jnp.concatenate(
                    [dq[:, 0:BQ], dq[:, BQ:]], axis=0)
            ds = ds_next
        ds_v[...] = ds

    def first_scores(i, carry):
        half = pl.ds(pl.multiple_of((i & 1) * (seq // 2), CK), seq // 2)
        s_v[i >> 1, half, :] = _dot(k_v[half, :], qt_v[i >> 1])
        width = 3 * 128
        cols = pl.ds(pl.multiple_of(jnp.minimum(early + i * width, 6 * d - width), 128), width)
        mod_v[:, cols] = _dot(silu_c, wmod_v[:, cols])
        k_all, k_blk = (
            jnp.concatenate([k[r + CK - AHEAD_KEYS:r + CK] for r in range(0, k.shape[0], CK)],
                            axis=0) for k in (k_v[...], k_v[rows(i), :]))
        for e in range(dh):
            kpre_v[i, e] = jnp.broadcast_to(k_blk[:, e:e + 1], (VPU_KEYS, 128))
        for u in range(n_grp // n_blk):
            g = i * (n_grp // n_blk) + u
            pre_v[g] = jnp.exp2(_dot(k_all, qt_v[g]))
        return carry

    assert n_blk == 2 * FWD_UNROLL == kpre_v.shape[0]
    cp_wmod_b.wait()
    jax.lax.fori_loop(0, n_blk, first_scores, 0)

    def block(b, carry):
        @pl.when(b == 0)
        def _():
            for cp in cp_late:
                cp.start()

        def fwd_body(i, carry):
            fwd_steps(i * FWD_UNROLL, range(FWD_UNROLL),
                      b * n_grp + (i + 1) * FWD_UNROLL, never_mask(i))
            return carry

        def fwd_tail(u, carry):
            fwd_steps(n_grp - FWD_UNROLL, [u])
            return carry

        last = jnp.where(b == n_blk - 1, 1, 0)
        jax.lax.fori_loop(0, n_grp // FWD_UNROLL - last, fwd_body, 0)
        jax.lax.fori_loop(0, last * FWD_UNROLL, fwd_tail, 0)

        @pl.when(b == 0)
        def _():
            for cp in cp_late:
                cp.wait()
            gate_dout(0)

        never = never_mask(b)[:, 0:128]
        g_ahead = jnp.minimum(b + 1, n_blk - 1) * n_grp
        todo = [(g, j) for g in range(n_grp) for j in range(kpre_v.shape[0])]

        def score_ahead(pieces):
            g, j = todo.pop(0)
            vpu = _VpuRows(kpre_v, qt_v, g_ahead + g, j)
            for i in range(pieces):
                yield vpu.partial((i + 1) * 2 * dh // pieces)
            pre_v[g, pl.ds(j * VPU_KEYS, VPU_KEYS), :] = jnp.exp2(vpu.result())

        def with_scores(name, x):
            count = AHEAD_PLAN[name]
            n_c = x.shape[1] // 128
            return _pin(x, never, [
                [acc for _ in range(count * (c + 1) // n_c - count * c // n_c)
                 for acc in score_ahead(AHEAD_PIECES)] for c in range(n_c)])

        ga, sb, cb, gb = modrow(2), modrow(3), modrow(4), modrow(5)
        dout = dout_v[rows(b), :].astype(F32)
        dm = dm_v[...]
        linv, o_heads = [], []
        for g in range(n_grp):
            linv_g = 1.0 / pv_v[g, dh:dh + 1, :]
            o_g = pv_v[g, 0:dh, :] * linv_g
            linv += [linv_g[:, 0:BQ], linv_g[:, BQ:]]
            o_heads += [o_g[:, 0:BQ], o_g[:, BQ:]]
        ot16 = jnp.concatenate(o_heads, axis=0).astype(BF16)
        dg_head = _dot(w2_v[0:DG_CUTS[0], :], dm, _NT)
        a = _dot(ot16, with_scores("a", wo_v[...]), _TN)
        x1 = x_v[rows(b), :].astype(F32) + ga * a
        stages = []
        x1hat, rstd1 = _layernorm(x1, stages)
        h2 = (x1hat * (1.0 + cb) + sb).astype(BF16)
        cuts = DG_CUTS + (w2_v.shape[0],)
        dgt = jnp.concatenate([dg_head] + [
            _dot(_pin_value(with_scores("dg", w2_v[lo:hi, :]), never, stage, band), dm, _NT)
            for lo, hi, stage, band in zip(cuts, cuts[1:], stages + [h2], (0, 32, 1))], axis=0)
        ut = _dot(with_scores("u", w1t_v[...]), h2, _NT)
        sig = _sigmoid(ut)
        gt = ut * sig
        dut = (dgt * (sig + gt * (1.0 - sig))).astype(BF16)
        gt = gt.astype(BF16)

        def wgrad(name, acc_ref, st_ref, lhs, rhs, spread=None, band=0):
            tot = _pin_value(with_scores(name, acc_ref[...]), never, spread, band)
            tot = tot + _dot(lhs, rhs)
            acc_ref[...] = tot
            st_ref[...] = tot.astype(BF16)

        wgrad("dw2", dw2_acc, dw2_s, gt, dm)
        gate_dout(jnp.minimum(b + 1, n_blk - 1))
        dh2 = _dot(dut, with_scores("dh2", w1t_v[...]), _TN)
        dx1 = dout + _layernorm_bwd(dh2 * (1.0 + cb), x1hat, rstd1)
        dx_acc[rows(b), :] = dx1
        da = (dx1 * ga).astype(BF16)
        mlp = _dot(gt, with_scores("mlp", w2_v[...]), _TN)
        out_s[rows(b), :] = (x1 + gb * mlp).astype(BF16)
        dmod_acc[:, 2 * d:3 * d] += _rowsum8(dx1 * a)
        dmod_acc[:, 3 * d:4 * d] += _rowsum8(dh2)
        dmod_acc[:, 4 * d:5 * d] += _rowsum8(dh2 * x1hat)
        dmod_acc[:, 5 * d:6 * d] += _rowsum8(dout * mlp)
        dot_full = _dot(with_scores("do", wo_v[...]), da, _NT)

        tails = []
        for hd in range(N_HEADS):
            g, cols = hd // 2, pl.ds((hd % 2) * BQ, BQ)
            do = dot_full[hd * dh:(hd + 1) * dh] * linv[hd]
            do = do.astype(BF16).astype(F32)
            nd = -jnp.sum(do * o_heads[hd], axis=0, keepdims=True)
            do = jnp.concatenate([do, _split_rows(nd)], axis=0)
            dot_v[g, :, cols] = do
            tails.append(do[DP - 8:])
        wgrad("dw1", dw1t_acc, dw1t_s, dut, h2, jnp.concatenate(tails, axis=0), 1)

        dp = _dot(v_v[keys(0), :], dot_v[0])
        ds_v[...] = (p_v[0, keys(0), :].astype(F32) * dp).astype(BF16)
        wgrad("dwo", dwo_acc, dwo_s, ot16, da)
        assert not todo
        cp_out(b).start()

        @pl.when(b == n_blk - 1)
        def _():
            for cp in cp_w_early:
                cp.start()

        def bwd_body(i, carry):
            bwd_steps(b, i * BWD_UNROLL, never_mask(i))
            return carry

        jax.lax.fori_loop(0, n_grp // BWD_UNROLL, bwd_body, 0)

        return carry

    jax.lax.fori_loop(0, n_blk, block, 0)

    r = jax.lax.broadcasted_iota(jnp.int32, (DP, seq), 0)
    dqt_v[d:d + DP, :] = jnp.where(r < dh, dkt_acc[...] * math.log(2.0), 0.0)
    dqt_v[d + DP:, :] = jnp.where(r < dh, dvt_acc[...], 0.0)

    dmod_acc[:, early:] = jnp.broadcast_to(
        jnp.sum(dmod_acc[:, early:], axis=0, keepdims=True), (8, 4 * d))

    def outer(part, row):
        col = jnp.concatenate([siluc_v[part, :]] * (row.shape[1] // 128), axis=1)
        return (col * row).astype(BF16)

    def inner(w, row):
        return _fold(w.astype(F32) * row)

    def finish_dx(b, carry):
        never = never_mask(b)[:, 0:128]
        lo, hi = DW_CUTS
        h = h_v[rows(b), :]
        dsilu = inner(wmod_v[mod_rows(b), early:], dmod_acc[0:1, early:])
        dwmod = outer(mod_rows(b), dmod_acc[0:1, early:])
        dsilu_v[mod_rows(b), :] = dsilu
        dwmod_s[mod_rows(b), early:] = dwmod
        stages = []
        xhat, rstd = _layernorm(x_v[rows(b), :].astype(F32), stages)

        def dw_rows(start, stop, spread=None, band=0):
            acc = _pin_value(dwt_acc[start:stop, :], never, spread, band)
            dwt_acc[start:stop, :] = acc + _dot(
                dqt_v[DW_SPLIT + start:DW_SPLIT + stop, rows(b)], h)

        dw_rows(0, lo, dsilu, 1)
        wt = _pin_value(wt_v[0:d + 2 * DP, :], never, stages[1], 32)
        wt = _pin_value(wt, never, jnp.concatenate(
            [dwmod[:, i:i + d] for i in range(0, 4 * d, d)], axis=0), 1)
        dq = dqt_v[:, rows(b)].astype(BF16).T
        dhh = jnp.concatenate([_dot(dq[:BQ // 2], wt_v[0:d + 2 * DP, :]),
                               _dot(dq[BQ // 2:], wt)], axis=0)
        dmod_acc[:, 0:d] += _rowsum8(dhh)
        dmod_acc[:, d:2 * d] += _rowsum8(dhh * xhat)
        dx = _layernorm_bwd(dhh * (1.0 + modrow(1)), xhat, rstd)
        dx = (dx_acc[rows(b), :] + dx).astype(BF16)
        dx_s[rows(b), :] = dx
        dw_rows(lo, hi)
        dw_rows(hi, d + 2 * DP - DW_SPLIT)
        cp_dx(b).start()
        cp_dwmod(b).start()
        return carry

    jax.lax.fori_loop(0, n_blk, finish_dx, 0)
    dmod = jnp.sum(dmod_acc[:, 0:early], axis=0, keepdims=True)
    dmod_acc[0:1, 0:early] = dmod
    dwkt_s[...] = dwt_acc[pl.ds(d - DW_SPLIT, dh), :].astype(BF16)
    dwvt_s[...] = dwt_acc[pl.ds(d - DW_SPLIT + DP, dh), :].astype(BF16)
    dw_rest = dwo_acc.at[0:DW_SPLIT]
    dw_rest[...] = jnp.zeros(dw_rest.shape, F32)
    for cp in cp_w_late:
        cp.start()

    def finish_dwq(i, carry):
        part = pl.ds(pl.multiple_of(2 * i * BQ, BQ), 2 * BQ)
        never = never_mask(i)[:, 0:128]
        quarter, strip = last_parts(i)
        dsilu = dsilu_v[quarter, :] + inner(wmod_v[quarter, 0:early], dmod_acc[0:1, 0:early])
        dwmod = outer(quarter, dmod_acc[0:1, 0:early])
        dsilu_v[quarter, :] = dsilu
        dwmod_s[quarter, 0:early] = dwmod
        dwq_s[:, strip] = dwt_acc[pl.ds(pl.multiple_of(i * 128, 128), 128), :].T.astype(BF16)
        dqt = _pin_value(dqt_v[0:DW_SPLIT, part], never, dsilu, 1)
        dw_rest[...] += _dot(_pin_value(dqt, never, dwmod, 1), h_v[part, :])
        for cp in cp_last(i):
            cp.start()
        return carry

    jax.lax.fori_loop(0, n_blk // 2, finish_dwq, 0)
    dwq_s[:, 0:DW_SPLIT] = dw_rest[...].T.astype(BF16)
    dsilu = jnp.sum(dsilu_v[...].T, axis=0, keepdims=True)
    dc_s[:, 0:d] = (dsilu * (sig_c + silu_c * (1.0 - sig_c)))[0:1].astype(BF16)
    for cp in cp_w_last:
        cp.start()

    for b in range(n_blk):
        cp_out(b).wait()
        cp_dx(b).wait()
        cp_dwmod(b).wait()
    for i in range(n_blk // 2):
        for cp in cp_last(i):
            cp.wait()
    for cp in cp_w_early + cp_w_late + cp_w_last:
        cp.wait()


@jax.jit
def pallas_adaLN_cond__grouped_kv_mqa__dense_activation_silu__prompt_kernel(
    A_x: jax.Array,
    A_wq: jax.Array,
    A_wk: jax.Array,
    A_wv: jax.Array,
    A_wo: jax.Array,
    B_x: jax.Array,
    B_w1: jax.Array,
    B_w2: jax.Array,
    c: jax.Array,
    w_mod: jax.Array,
    grad_out: jax.Array,
):
    del B_x
    _, seq, d = A_x.shape
    dh = d // N_HEADS
    f = B_w1.shape[1]
    n_grp = N_HEADS // 2
    n_blk = seq // BQ

    n_pre = seq // CK * AHEAD_KEYS

    def vmem(shape, dtype):
        return pltpu.VMEM(shape, dtype)

    out_shapes = [(seq, d), (seq, d), (d, d), (dh, d), (dh, d), (d, d), (f, d), (f, d),
                  (1, d), (d, 6 * d)]
    big_shapes = [s for s in out_shapes if s[0] > dh]
    scratch = (
        [vmem(s, BF16) for s in [(dh, d)] * 4 + [(1, 1024)] * 2 + big_shapes]
        + [
            vmem((2 * DP, d), F32),
            vmem((8, 6 * d), F32),
            vmem((16, 6 * d), F32),
            vmem((d + 64 - DW_SPLIT, d), F32),
            vmem((d + 64, d), BF16),
            vmem((seq, d), BF16),
            vmem((seq, DP), F32),
            vmem((seq, DP), F32),
            vmem((DP, seq), F32),
            vmem((DP, seq), F32),
            vmem((seq // CK, dh, VPU_KEYS, 128), F32),
            vmem((n_pre // VPU_KEYS, dh, VPU_KEYS, 128), F32),
            vmem((seq // CK, dh, VPU_KEYS, 128), F32),
            vmem((n_grp, n_pre, 2 * BQ), F32),
            vmem((16, BQ), F32),
            vmem((d, 128), F32),
            vmem((n_blk * n_grp, DP, 2 * BQ), F32),
            vmem((n_grp, DP, 2 * BQ), F32),
            vmem((n_grp, DP, 2 * BQ), F32),
            vmem((BQ, d), BF16),
            vmem((d + 2 * DP, seq), F32),
            vmem((FWD_UNROLL, seq, 2 * BQ), F32),
            vmem((n_grp, seq, 2 * BQ), BF16),
            vmem((CK, 2 * BQ), BF16),
            vmem((seq, d), F32),
            vmem((DP, seq), F32),
            vmem((DP, seq), F32),
            vmem((d, d), F32),
            vmem((f, d), F32),
            vmem((f, d), F32),
        ]
        + [vmem((d, 128), F32)]
        + [vmem(s, BF16) for s in [(d, d), (f, d), (f, d)]]
        + [
            pltpu.SemaphoreType.DMA((10,)),
            pltpu.SemaphoreType.DMA((n_blk,)),
            pltpu.SemaphoreType.DMA((n_blk,)),
            pltpu.SemaphoreType.DMA((n_blk,)),
            pltpu.SemaphoreType.DMA((n_blk,)),
            pltpu.SemaphoreType.DMA((15,)),
        ]
    )
    hbm = pl.BlockSpec(memory_space=pl.ANY)
    out, dx, dwq, dwkt, dwvt, dwo, dw1t, dw2, dc, dwmod = pl.pallas_call(
        _kernel,
        out_shape=[jax.ShapeDtypeStruct(s, BF16) for s in out_shapes],
        in_specs=[hbm] * 10,
        out_specs=[hbm] * 10,
        scratch_shapes=scratch,
        compiler_params=pltpu.CompilerParams(vmem_limit_bytes=127 * 1024 * 1024),
        name="adaln_mqa_mlp_fwd_bwd",
    )(
        A_x.reshape(seq, d), A_wq, A_wk.T, A_wv.T, A_wo, B_w1.T, B_w2, c, w_mod,
        grad_out.reshape(seq, d),
    )
    return (
        out.reshape(A_x.shape), dx.reshape(A_x.shape), dwq, dwkt.T, dwvt.T, dwo,
        dw1t.T, dw2, dc, dwmod,
    )
```
